```python
import os as _os
_os.environ.setdefault("JAX_PLATFORMS", "cpu")
import jax
import jax.numpy as jnp

def _softmax(x, axis=-1):
    return jax.nn.softmax(x, axis=axis)
def _gelu(x):
    return jax.nn.gelu(x, approximate=True)
def _silu(x):
    return jax.nn.silu(x)
def _sigmoid(x):
    return jax.nn.sigmoid(x)
def _layernorm(x, axis=-1, eps=1e-5):
    m = jnp.mean(x, axis=axis, keepdims=True)
    v = jnp.var(x, axis=axis, keepdims=True)
    return (x - m) / jnp.sqrt(v + eps)
def _scatter_add(tgt, idx, src, axis=0):
    return tgt.at[idx].add(src)
def _segment_sum(src, seg, n):
    return jax.ops.segment_sum(src, seg, n)
class _Rng:
    def __init__(self, key):
        self._k = key
    def _next(self):
        self._k, sub = jax.random.split(self._k)
        return sub
    def normal(self, shape):
        return jax.random.normal(self._next(), shape, dtype=jnp.bfloat16)
    def randint(self, lo, hi, shape):
        return jax.random.randint(self._next(), shape, lo, hi, dtype=jnp.int32)
    def uniform(self, shape, lo=0.0, hi=1.0):
        return jax.random.uniform(self._next(), shape, jnp.bfloat16, lo, hi)
    def permutation(self, n):
        return jax.random.permutation(self._next(), n)


kernel_name = 'standalone__mixer_token_mlp__sampling'

def setup_inputs():
    _rng = _Rng(jax.random.key(int.from_bytes(__import__("os").urandom(4), "little")))
    _w = (lambda a: (lambda t: t.astype(jnp.bfloat16) if jnp.issubdtype(t.dtype, jnp.floating) else t)(jnp.asarray(a)))
    B, S, D, F = 32, 16, 1024, 3584
    return {
        "x": _w((lambda *s: _rng.normal(s) * 0.05)(B, S, D)),
        "w1": _w((lambda *s: _rng.normal(s) * 0.05)(S, F) * (S ** -0.5)),
        "b1": _w((lambda *s: _rng.normal(s) * 0.05)(F) * 0.02),
        "w2": _w((lambda *s: _rng.normal(s) * 0.05)(F, S) * (F ** -0.5)),
        "b2": _w((lambda *s: _rng.normal(s) * 0.05)(S) * 0.02),
    }

def reference(x, w1, b1, w2, b2):
    B, S, D = x.shape
    h = _layernorm(x, axis=-1)
    u = jnp.einsum("bsd,sf->bdf", h, w1) + b1
    u = _gelu(u)
    y = jnp.einsum("bdf,fs->bds", u, w2) + b2
    return (lambda x, *d: x.transpose(*d))(y, 0, 2, 1)
```

```python
import functools
import numpy as np
import jax, jax.numpy as jnp
from jax import lax
from jax.experimental import pallas as pl
from jax.experimental.pallas import tpu as pltpu
import ml_dtypes

C1 = float(np.sqrt(2 / np.pi)); C2 = C1 * 0.044715
KS = C2 ** (1.0 / 3.0)
CC = C1 / KS
K_HI = float(np.float32(KS).astype(ml_dtypes.bfloat16)); K_LO = float(np.float32(KS - K_HI).astype(ml_dtypes.bfloat16))
f32 = jnp.float32; bf16 = jnp.bfloat16; u32 = jnp.uint32
pk = lambda a: pltpu.bitcast(a, u32)
upk = lambda a: pltpu.bitcast(a, bf16)
S = 16; DC = 512

def act(v):
    return v * jnp.tanh(v * (CC + v * v))

def left_factors(a, lv):
    if lv == 0: return [a[0]]
    m, k = a.shape[0] // 2, a.shape[1] // 2
    a11, a12, a21, a22 = a[:m, :k], a[:m, k:], a[m:, :k], a[m:, k:]
    s1 = a21 + a22; s2 = s1 - a11
    return [z for y in (a11, a12, a12 - s2, a22, s1, s2, a11 - a21) for z in left_factors(y, lv - 1)]

def right_factors(b, lv):
    if lv == 0: return [b[0]]
    n, k = b.shape[0] // 2, b.shape[1] // 2
    b11, b21, b12, b22 = b[:n, :k], b[:n, k:], b[n:, :k], b[n:, k:]
    t1 = b12 - b11; t2 = b22 - t1
    return [z for y in (b11, b21, b22, b21 - t2, t1, t2, b22 - b12) for z in right_factors(y, lv - 1)]

def bias_factors(c, lv):
    if lv == 0: return {0: c[0]}
    m = len(c) // 2
    lo = bias_factors(c[:m], lv - 1); hi = bias_factors([y - x for x, y in zip(c[:m], c[m:])], lv - 1)
    return {**lo, **{6 * 7 ** (lv - 1) + i: v for i, v in hi.items()}}

def combine(p):
    p1 = p(0); yield (0, 0), p1 + p(1)
    u2 = p1 + p(5); u3 = u2 + p(6)
    yield (1, 0), u3 + p(3)
    p5 = p(4); yield (1, 1), u3 + p5
    yield (0, 1), (u2 + p5) + p(2)

def kern(x_hbm, w1_hbm, b1_hbm, w2t_hbm, b2_hbm, o_hbm,
         x_ref, w1_ref, b1_ref, w2t_ref, b2_ref, o_ref, lhs_ref, b2s_ref, ha_ref, hf_ref, wt_ref, mean_ref, rstd_ref, carry_ref, isem, osem, *ht_refs,
         J, L, NV, LV, AHEAD, HEAD, SKIP, MINC, XCUT, P0, TC, HC, HPOS, VEND, BP, PS, PE):
    B, _, D = x_ref.shape; F = w1_ref.shape[1]
    nd = D // DC; nf = F // 128; njob = B * nd
    W2 = 8 * nf; LINB = W2 + nf; JUNK = LINB + 1; TMP = JUNK + 1; PARK = TMP + 56
    vt = list(range(nf - VEND - NV, nf - VEND))
    G = 2 ** LV; NP = 7 ** LV; KI = S // G; nsb = 2 * NV // G
    buf = [n % 2 for n in range(J)]
    if J % 2: buf[-1] = 2

    cuts = [0] + list(XCUT) + [B]
    cps = [pltpu.make_async_copy(s_, d_, isem.at[i]) for i, (s_, d_) in enumerate(
        [(x_hbm.at[0:1], x_ref.at[0:1]), (w1_hbm, w1_ref), (b1_hbm, b1_ref), (w2t_hbm, w2t_ref), (b2_hbm, b2_ref)]
        + [(x_hbm.at[a:b], x_ref.at[a:b]) for a, b in zip(cuts[1:-1], cuts[2:])])]

    slots = []; due = []
    for n in range(4):
        stream = [(j, p) for j in range(nf) for p in range(7, 0 if (n and j in vt) else -1, -1)]
        stream.insert(len(stream) - 4, ("lin", 0))
        for i, (j, p) in enumerate(stream):
            slots.append(("x", n, j, p))
            if j != "lin" and (i + 1 == len(stream) or stream[i + 1][0] not in (j, "lin")):
                due.append((len(slots) + L, ("y", n, j)))
            while due and due[0][0] <= len(slots):
                slots.append(due.pop(0)[1])
    ends = [i + 1 for i, s in enumerate(slots) if s[0] == "y" and s[2] == nf - 1]
    first_period = slots[:ends[0]]
    period = [(s[0], s[1] - 1) + s[2:] for s in slots[ends[0]:ends[1]]]
    assert period == [(s[0], s[1] - 2) + s[2:] for s in slots[ends[1]:ends[2]]]
    keys = [(0,) + s[2:] for s in period if s[:2] == ("x", 1)]

    def job_slice(job):
        if isinstance(job, int): return job // nd, pl.ds((job % nd) * DC, DC)
        return lax.shift_right_logical(job, 1), pl.ds(pl.multiple_of((job & 1) * DC, DC), DC)

    def stats(b):
        x = x_ref[b].astype(f32)
        m = jnp.mean(x, axis=-1, keepdims=True)
        xc = x - m
        r = jnp.broadcast_to(lax.rsqrt(jnp.mean(xc * xc, axis=-1, keepdims=True) + 1e-5) * KS, (S, 128))
        mean_ref[b] = jnp.broadcast_to(m, (S, 128)); rstd_ref[b] = r
        return r[8:]

    def normalize(job, slot, z):
        b, cols = job_slice(job)
        h = ((x_ref[b, :, cols].astype(f32) - jnp.tile(mean_ref[b], (1, 4))) * jnp.tile(rstd_ref[b], (1, 4))).astype(bf16)
        ha_ref[slot] = pk(h)
        hf = h.astype(f32)
        for t in range(4): hf_ref[t + z] = hf[:, t * 128:(t + 1) * 128]
        return hf[8:, 384:]

    def h_items(ht_ref, z):
        for c in range(4 // G):
            for i in range(KI):
                rows = [[jnp.broadcast_to(hf_ref[c * G + t, s * KI + i:s * KI + i + 1, :], (8, 128)) for s in range(G)] for t in range(G)]
                fs = right_factors(jnp.stack([jnp.stack(r) for r in rows]), LV)
                for n, v in enumerate(fs):
                    ht_ref[c + z, n * KI + i] = v[0]
                    yield HC, None, v[0]
    nh = 4 // G * KI * NP

    def v_items(ht_ref):
        bias = list(bias_factors(list(range(G)), LV))
        H = G // 2
        def phase_a(u, sb, c):
            def prod(n):
                r = wt_ref[sb, NP * KI + bias.index(n)] if n in bias else None
                for i in range(n * KI, (n + 1) * KI, TC):
                    p = wt_ref[sb, i:i + TC] * ht_ref[c, i:i + TC]
                    for e in range(TC): r = p[e] if r is None else r + p[e]
                return r
            if LV == 0:
                yield 37, PARK + sb * 4 + c, act(prod(0))
            for o in range(7 if LV else 0):
                if LV == 1: yield 15 + (o in bias), TMP + (u % 2) * 28 + o * 4, prod(o)
                else:
                    for cost, (key, v) in zip((15, 24, 8, 9), combine(lambda i: prod(7 * o + i))):
                        yield cost + 0.5 * (7 * o in bias), TMP + (u % 2) * 28 + o * 4 + 2 * key[0] + key[1], v
        def phase_b(u, sb, c):
            for r in range(H):
                for t in range(H):
                    outs = [(k, act(v)) for k, v in combine(lambda o: pltpu.bitcast(lhs_ref[TMP + (u % 2) * 28 + o * 4 + 2 * r + t], f32))]
                    yield [(BP[2], None, None)]
                    yield [((27 - BP[2]) / 4, PARK + (sb * G + k[0] * H + r) * 4 + c * G + k[1] * H + t, v) for k, v in outs]
        pending = iter(())
        for u, (sb, c) in enumerate((sb, c) for sb in range(nsb) for c in range(4 // G)):
            for n, item in enumerate(phase_a(u, sb, c)):
                yield item
                if n % 7 in BP[:2]: yield from next(pending, [])
            assert next(pending, None) is None
            pending = phase_b(u, sb, c)
        for its in pending: yield from its

    def merged(main, extra, start, every):
        done = 0.0; nxt = start
        for item in main:
            yield item
            done += item[0]
            while done >= nxt:
                e = next(extra, None)
                if e is None: nxt = float("inf")
                else: yield e; nxt += every
        yield from extra

    def run_period(plan, job, slot, g, items, total, z, lhs_of, head=0.0, skip=0, end=0):
        acc = jnp.tile(b2s_ref[...], (1, 4)) if plan is period else None
        run = []; done = 0.0; since = 0.0; parked = set()
        row = lax.broadcasted_iota(jnp.int32, (S, DC), 0)
        cst = jnp.where(row == 0, K_HI, jnp.where(row == 1, K_LO, 0.0)).astype(bf16)
        def flush():
            nonlocal acc
            if not run: return
            h = upk(ha_ref[(slot + run[0][0][1]) % J])
            rhs = jnp.concatenate([h, cst] + [h] * any(s[2] == "lin" for s, _ in run), axis=0)
            lhs = upk(jnp.concatenate([v for _, v in run], axis=0))
            u = jnp.dot(lhs[:, :rhs.shape[0]], rhs, preferred_element_type=f32)
            for n, (s, _) in enumerate(run):
                ub = u[16 * n:16 * n + 16]
                if s[2] == "lin": acc = acc + ub
                else: g[s[1:]] = act(ub)
            run.clear()
        for n, s in enumerate(plan):
            target = (total - head) * min(1.0, max(0, n + 1 - skip) / (len(plan) - skip - end)) + head * min(1.0, max(n + 1 - skip, 0) / 6)
            need = []
            if n + AHEAD < len(plan) and plan[n + AHEAD][0] == "y" and plan is period and plan[n + AHEAD][2] in vt:
                j = plan[n + AHEAD][2]
                need = [[PARK + (2 * vt.index(j) + q) * 4 + t for t in range(4)] for q in range(2)]
            while done < target - 1e-6 or any(i not in parked for r in need for i in r) or n == len(plan) - 1 - end:
                it_ = next(items, None)
                if it_ is None: break
                cost, where, v = it_
                done += cost; since += cost
                if where is not None: parked.add(where)
                if v is not None and (where is not None or since >= MINC):
                    lhs_ref[(JUNK if where is None else where) + z] = pk(v); since = 0.0
            if need:
                g[0, j, 0] = jnp.concatenate([jnp.concatenate([pltpu.bitcast(lhs_ref[i], f32) for i in r], axis=1) for r in need], axis=0)
            if s[0] == "x":
                if run and run[0][0][1] != s[1]: flush()
                run.append((s, lhs_of(LINB if s[2] == "lin" else 8 * s[2] + s[3])))
            else:
                flush()
                p = jnp.dot(upk(lhs_of(W2 + s[2])), jnp.concatenate([g.pop((0, s[2], p)) for p in range(8)], axis=0), preferred_element_type=f32)
                if acc is None: lhs_ref[JUNK + z] = pk(p[:8, :128])
                acc = p if acc is None else acc + p
        b, cols = job_slice(job)
        if plan is not period: acc = acc + jnp.tile(b2s_ref[...], (1, 4))
        o_ref[b, :, cols] = (acc * (0.5 / KS)).astype(o_ref.dtype)
        return {(0,) + k[1:]: v for k, v in g.items()}

    def save(g):
        for i, k in enumerate(keys): carry_ref[i] = g[k]

    def first(z):
        for c in cps: c.start()
        cps[0].wait()
        stats(0); normalize(0, J - 1, z)
        for c in cps[1:5]: c.wait()
        b1 = b1_ref[...].astype(f32)
        row = lax.broadcasted_iota(jnp.int32, (8, 128), 0)
        built = set()
        def tile(j):
            if j not in built and j < nf:
                built.add(j)
                w = w1_ref[:, j * 128:(j + 1) * 128].astype(f32)
                bb = jnp.where(row < 2, jnp.broadcast_to(b1[j:j + 1, :], (8, 128)), 0.0)
                a = jnp.concatenate([w, bb, jnp.zeros((128 - S - 8, 128), f32)], axis=0).T
                lhs_ref[pl.ds(8 * j + z, 8)] = pk(a.astype(bf16)).reshape(8, 8, 128)
                lhs_ref[W2 + j + z] = pk(w2t_ref[:, j * 128:(j + 1) * 128])
        def lhs_first(i):
            if i == 8 * (nf - 3):
                for j in range(nf): tile(j)
                M = jnp.dot(w2t_ref[...], upk(lhs_ref[:W2].reshape(4 * F // 8, 128)), preferred_element_type=f32)
                r = lax.broadcasted_iota(jnp.int32, (S, S), 0); c = lax.broadcasted_iota(jnp.int32, (S, S), 1)
                b2 = jnp.sum(jnp.where(r == c, jnp.broadcast_to(b2_ref[...].astype(f32), (S, S)), 0.0), axis=1, keepdims=True)
                b2s_ref[...] = jnp.broadcast_to((2.0 * b2 + M[:, S:S + 1]) * KS, (S, 128))
                lane = lax.broadcasted_iota(jnp.int32, (S, 128), 1)
                Mhi = M.astype(bf16).astype(f32)
                built.add(("lin", pk((jnp.where(lane < S, Mhi, 0.0) + pltpu.roll(M - Mhi, 2 * S, 1)).astype(bf16)).reshape))
            if i == LINB: lhs_ref[LINB + z] = [e for e in built if isinstance(e, tuple)][0][1](8, 128)
            elif i < W2: tile(i // 8)
            return lhs_ref[i]
        def setup_items():
            cols = {}
            def col(gi, s):
                j = vt[gi // 2]
                if (j, s) not in cols:
                    tile(j)
                    if j not in cols: cols[j] = lhs_ref[8 * j]
                    cols[j, s] = upk(jnp.broadcast_to(cols[j][:, s:s + 1], (8, 128))).astype(f32)
                return cols[j, s][8 * (gi % 2):8 * (gi % 2) + 8]
            def w_items(sbs):
                for i in range(KI):
                    for sb in sbs:
                        fs = left_factors(jnp.stack([jnp.stack([col(sb * G + r, s * KI + i) for s in range(G)]) for r in range(G)]), LV)
                        for n, v in enumerate(fs): wt_ref[sb, n * KI + i] = v[0]
                for sb in sbs:
                    for n, v in enumerate(bias_factors([col(sb * G + r, S) * KS for r in range(G)], LV).values()):
                        wt_ref[sb, NP * KI + n] = v
                return v
            yield P0, None, normalize(1, 0, z)
            hs = h_items(ht_refs[0], z)
            nb = 1; st = 2 if LV == 0 else 1; late = []
            for sb in range(0, nsb, st):
                late.append(w_items(range(sb, sb + st)))
                yield st * (NP * KI + G), None, (late.pop(0) if len(late) > PS else None)
                for _ in range(-(-nh * st // nsb)):
                    e = next(hs, None)
                    if e is not None: yield e
                while nb < 1 + (B - 1) * (sb + st) // nsb:
                    if nb in cuts: cps[4 + cuts.index(nb)].wait()
                    yield 80.0, None, stats(nb); nb += 1
        save(run_period(first_period, 0, J - 1, {}, setup_items(), P0 + nsb * (NP * KI + G) + 80.0 * (B - 1) + nh * HC, z, lhs_first, skip=4, end=PE))

    def out_copy(job):
        b, cols = job_slice(job)
        return pltpu.make_async_copy(o_ref.at[b, :, cols], o_hbm.at[b, :, cols], osem)

    def body(it, carry):
        z = lax.shift_right_logical(it, 20)
        @pl.when(it == 0)
        def _(): first(z)
        @pl.when(it > 0)
        def _():
            g = {k: carry_ref[i] for i, k in enumerate(keys)}
            for n in range(J):
                job = 1 + (it - 1) * J + n; nxt = jnp.minimum(job + 1, njob - 1)
                out_copy(job - 1).start()
                def extra():
                    yield 36.0, None, normalize(nxt, (n + 1) % J, z)
                    yield from h_items(ht_refs[buf[(n + 1) % J]], z)
                vcost = NV * 8 * (5 + (32, 28.5, 26.5)[LV])
                items = merged(v_items(ht_refs[buf[n]]), extra(), HPOS * vcost, (0.95 - HPOS) * vcost / nh)
                g = run_period(period, job, n, g, items, 36.0 + nh * HC + vcost, z, lambda i: lhs_ref[i], HEAD if n == 0 else 0.0, SKIP if n == 0 else 0)
            save(g)
        return carry
    lax.fori_loop(0, 1 + (njob - 1) // J, body, 0)
    out_copy(njob - 1).start()
    pltpu.make_async_copy(o_ref, o_hbm, osem).wait()

DEF = dict(J=3, L=10, NV=20, LV=0, AHEAD=3, HEAD=100.0, SKIP=3, MINC=3, XCUT=(1, 8), P0=400.0, TC=4, HC=1.0, HPOS=0.1, VEND=0, BP=(0, 3, 27), PS=2, PE=12)
def make(flags={"XLA_TPU_EVENLY_DISTRIBUTE_CRITICAL_NODES": True}, **kw):
    p = {**DEF, **kw}
    p = {k: tuple(v) if isinstance(v, list) else v for k, v in p.items()}
    @jax.jit
    def f(x, w1, b1, w2, b2):
        B, _, D = x.shape; F = w1.shape[1]
        LV, NV, J, L = p["LV"], p["NV"], p["J"], p["L"]; G = 2 ** LV
        args = (x, w1, b1.reshape(F // 128, 128), w2.T, b2.reshape(1, S))
        hbm = pl.BlockSpec(memory_space=pltpu.HBM)
        return pl.pallas_call(
            functools.partial(kern, **p),
            out_shape=jax.ShapeDtypeStruct(x.shape, x.dtype),
            in_specs=[hbm] * 5, out_specs=hbm,
            scratch_shapes=[pltpu.VMEM(a.shape, a.dtype) for a in args] + [pltpu.VMEM(x.shape, x.dtype),
                            pltpu.VMEM((9 * F // 128 + 58 + 8 * NV, 8, 128), u32), pltpu.VMEM((S, 128), f32),
                            pltpu.VMEM((J, S // 2, DC), u32), pltpu.VMEM((4, S, 128), f32),
                            pltpu.VMEM((2 * NV // G, 7 ** LV * S // G + G, 8, 128), f32),
                            pltpu.VMEM((B, S, 128), f32), pltpu.VMEM((B, S, 128), f32), pltpu.VMEM((L + 2, S, DC), f32),
                            pltpu.SemaphoreType.DMA((5 + len(p["XCUT"]),)), pltpu.SemaphoreType.DMA(())]
                           + [pltpu.VMEM((4 // G, 7 ** LV * S // G, 8, 128), f32)] * 3,
            compiler_params=pltpu.CompilerParams(vmem_limit_bytes=96 * 2**20, flags=flags),
        )(*args)
    return f

_f = make()

@jax.jit
def pallas_standalone__mixer_token_mlp__sampling_kernel(x, w1, b1, w2, b2):
    return _f(x, w1, b1, w2, b2)
```

```python
import functools

import jax
import jax.numpy as jnp
import numpy as np
from jax import lax
from jax.experimental import pallas as pl
from jax.experimental.pallas import tpu as pltpu

f32, bf16, u32 = jnp.float32, jnp.bfloat16, jnp.uint32

EPS = 1e-5
MIN_BIAS = -1.0
K = float((0.044715 * np.sqrt(2 / np.pi)) ** (1 / 3))
C = float(np.sqrt(2 / np.pi)) / K
K_HI = float(np.round(K * 512) / 512)
K_LO = K - K_HI

S = 16
COLS = 512
TILES = COLS // 128
VPU_BLOCKS = ((22, 23, 23, 23), (23, 23, 23, 23, 23))
LAG = 10
NH = 7 * TILES // 2
TERMS = 4
COSTS = (20, 40, 40, 34)
AHEAD, START, HEAD_OPS, END, STATS_AT, STATS_STEP, GATE = 2, 10, 100, 1, 16, 2, 9
TABLE_FROM, TABLE_SPAN = 0.1, 0.8
SETUP_START, SETUP_OPS, SETUP_END, SETUP_GATE, SETUP_STEP, TRANSPOSE_AHEAD = 36, 300, 8, 14, 4, 5


def _words(a):
    return pltpu.bitcast(a, u32)


def _act(v):
    return v * jnp.tanh(v * (C + v * v))


def _lanes(a, t):
    return a[:, 128 * t:128 * (t + 1)]


def _plan(nf):
    counts = (0,) + tuple(sum(map(list, VPU_BLOCKS), [])) + (0,)
    slots, due = [], []
    for n, count in enumerate(counts):
        first_vpu = nf - count
        for j in range(nf):
            blocks = list(range(7, 0 if j >= first_vpu else -1, -1))
            if j == nf - 1:
                blocks.insert(len(blocks) - 3, "linear")
            for p in blocks:
                slots.append(("x", n, j, p))
                if p == blocks[-1]:
                    due.append((len(slots) + LAG, ("y", n, j)))
                while due and due[0][0] <= len(slots):
                    slots.append(due.pop(0)[1])
    ends = [0] + [i + 1 for i, s in enumerate(slots) if s[0] == "y" and s[2] == nf - 1]
    return [[(s[0], s[1] - n) + s[2:] for s in slots[ends[n]:ends[n + 1]]] for n in range(len(counts) - 1)]


def _kernel(x_hbm, w1_hbm, b1_hbm, w2t_hbm, b2_hbm, o_hbm,
            x_ref, w1_ref, b1_ref, w2t_ref, b2_ref, o_ref,
            seq, acc0_ref, stat_ref, wcol_ref, carry_ref, k_ref, hrow_ref, split_ref, in_sem, out_sem, *h_refs):
    B, _, D = o_ref.shape
    F = w1_ref.shape[1]
    nf, njobs, nvpu = F // 128, B * D // COLS, max(map(max, VPU_BLOCKS))
    sizes = [len(v) for v in VPU_BLOCKS]
    cycle = sum(sizes)
    slots = (range(sizes[0]), range(sizes[0], cycle))
    steps = 2 * ((njobs - 1) // cycle) + ((njobs - 1) % cycle > 0)
    hsplat_refs, hmxu_refs = h_refs[:cycle], h_refs[cycle:]
    W2 = 8 * nf
    LINEAR = W2 + nf
    SPARE = LINEAR + 1
    PARK = SPARE + 3
    first_period, *periods = _plan(nf)
    carried = [("x", 0) + s[2:] for s in periods[-1] if s[:2] == ("x", 1)]
    for plan in (first_period, periods[sizes[0] - 1]):
        assert carried == [("x", 0) + s[2:] for s in plan if s[:2] == ("x", 1)]

    early = (cycle + sizes[0]) // 2 + 1
    late = (njobs - sizes[(steps - 1) % 2]) // 2
    loads = [pltpu.make_async_copy(src, dst, in_sem.at[i]) for i, (src, dst) in enumerate([
        (x_hbm.at[:early], x_ref.at[:early]), (w1_hbm, w1_ref), (b1_hbm, b1_ref),
        (w2t_hbm, w2t_ref), (b2_hbm, b2_ref), (x_hbm.at[early:], x_ref.at[early:])])]
    stores = [pltpu.make_async_copy(o_ref.at[a:b], o_hbm.at[a:b], out_sem.at[i])
              for i, (a, b) in enumerate([(0, late), (late, B)])]

    def job_slice(job):
        if isinstance(job, int):
            return job // 2, pl.ds(job % 2 * COLS, COLS)
        return lax.shift_right_logical(job, 1), pl.ds(pl.multiple_of((job & 1) * COLS, COLS), COLS)

    def moments(means, variances):
        centred = [x_ref[b].astype(f32) - jnp.tile(stat_ref[b], (1, D // 128)) for b in variances]
        out = []
        for i, v in [(b, x_ref[b].astype(f32)) for b in means] + [(B + b, d * d) for b, d in zip(variances, centred)]:
            out.append(jnp.broadcast_to(jnp.mean(v, axis=-1, keepdims=True), (S, 128)))
            stat_ref[i] = out[-1]
        return out

    def normalize(job):
        b, cols = job_slice(job)
        scale = lax.rsqrt(stat_ref[B + b] + EPS) * K
        centred = x_ref[b, :, cols].astype(f32) - jnp.tile(stat_ref[b], (1, TILES))
        return (centred * jnp.tile(scale, (1, TILES))).astype(bf16).astype(f32)

    def park_h(h, slot, z):
        hmxu_refs[slot][z] = h
        for c in range(TILES // 2):
            b11, b21, b12, b22 = (_lanes(h, 2 * c + i // 2)[8 * (i % 2):8 * (i % 2) + 8] for i in range(4))
            t1 = b12 - b11
            t2 = b22 - t1
            for i, v in enumerate((b11, b21, b22, b21 - t2, t1, t2, b22 - b12)):
                hrow_ref[1 + NH * slot + 7 * c + i + z] = v
        yield 0, None, None

    def publish_h(slot, z, ops=0):
        for i in range(NH):
            yield ops, "gate", None
            rows = hrow_ref[1 + NH * slot + i]
            for r in range(8):
                if ops:
                    start = pl.multiple_of(8 * (8 * i + r + z), 8)
                    hsplat_refs[slot][pl.ds(start, 8), :] = jnp.broadcast_to(rows[r:r + 1], (8, 128))
                else:
                    hsplat_refs[slot][pl.ds(z + (64 * i + r), 8, stride=8), :] = rows

    def vpu_rows(slot, count):
        for block in range(nvpu - count, nvpu):
            for c in range(TILES // 2):
                def add(v, i):
                    for s in range(8 * i, 8 * (i + 1), TERMS):
                        w = wcol_ref[block, s:s + TERMS]
                        h = hsplat_refs[slot][8 * (56 * c + s):8 * (56 * c + s + TERMS), :]
                        p = jnp.sum(w * h.reshape(TERMS, 8, 128), axis=0)
                        v = p if v is None else v + p
                    return v
                row = PARK + 2 * TILES * block + 2 * c
                p1 = add(wcol_ref[block, 56], 0)
                yield COSTS[0], row, _act(add(None, 1) + p1)
                u2 = add(None, 5) + p1
                u3 = add(wcol_ref[block, 57], 6) + u2
                yield COSTS[1], row + TILES, _act(add(None, 3) + u3)
                p5 = add(None, 4)
                yield COSTS[2], row + 1, _act(add(None, 2) + (u2 + p5))
                yield COSTS[3], row + TILES + 1, _act(u3 + p5)

    def run_period(plan, job, h_slots, acts, work, target, z, lhs, end, by_slot):
        acc = jnp.tile(acc0_ref[0], (1, TILES))
        k_rows = jnp.tile(k_ref[...], (1, TILES))
        run, results, parked, done = [], {}, set(), 0

        def first_matmul():
            nonlocal acc
            h = hmxu_refs[h_slots[plan[run[0][0]][1]]][0]
            rhs = jnp.concatenate([h, k_rows] + [h for n, _ in run if plan[n][3] == "linear"], axis=0)
            rows = pltpu.bitcast(jnp.concatenate([w for _, w in run], axis=0), bf16)
            v = jnp.dot(rows[:, :rhs.shape[0]], rhs, preferred_element_type=f32)
            g = _act(v)
            for i, (n, _) in enumerate(run):
                results[n] = functools.partial(lax.slice, v, (16 * i, 0), (16 * i + 8, 128))
                if plan[n][3] == "linear":
                    acc = acc + v[16 * i:16 * (i + 1)]
                else:
                    acts[plan[n][1:]] = g[16 * i:16 * (i + 1)]
            run.clear()

        for n, s in enumerate(plan):
            by_slot(n, results)
            soon = plan[min(n + AHEAD, len(plan) - 1)]
            fetch = n + AHEAD < len(plan) and soon[0] == "y" and ("x", 0, soon[2], 0) not in plan + carried
            base = PARK + 2 * TILES * (soon[2] - nf + nvpu)
            last = n == len(plan) - 1 - end
            while last or done < target(n) - 1e-6 or (fetch and base + 2 * TILES - 1 not in parked):
                ops, row, value = next(work, (None, None, None))
                if ops is None:
                    break
                done += ops
                if row == "gate":
                    hrow_ref[z] = stat_ref[2 * B + z, :8] = results[max(m for m in results if m <= n - GATE)]()
                elif value is not None:
                    parked.add(row)
                    seq[row + z] = _words(value)
            if fetch:
                halves = [jnp.concatenate([seq[base + TILES * q + t] for t in range(TILES)], axis=1) for q in range(2)]
                acts[0, soon[2], 0] = pltpu.bitcast(jnp.concatenate(halves, axis=0), f32)
            if s[0] == "x":
                if run and plan[run[0][0]][1] != s[1]:
                    first_matmul()
                run.append((n, lhs(LINEAR if s[3] == "linear" else 8 * s[2] + s[3])))
            else:
                first_matmul()
                tile = jnp.concatenate([acts.pop((0, s[2], p)) for p in range(8)], axis=0)
                y = jnp.dot(pltpu.bitcast(lhs(W2 + s[2]), bf16), tile, preferred_element_type=f32)
                acc = acc + y
                results[n] = functools.partial(lax.slice, y, (0, 0), (8, 128))
        b, cols = job_slice(job)
        o_ref[b, :, cols] = (acc * (0.5 / K)).astype(o_ref.dtype)
        return {(0,) + key[1:]: v for key, v in acts.items()}

    def ramp(total, first, last):
        return lambda n: total * min(1.0, max(0, n + 1 - first) / (last - first))

    def first_job(z):
        for copy in loads[:-1]:
            copy.start()
        row = lax.broadcasted_iota(jnp.int32, (8, 128), 0)
        k_ref[...] = jnp.where(row == 0, K_HI, jnp.where(row == 1, K_LO, 0.0))
        for copy in loads[:-1]:
            copy.wait()
        moments([0], [])
        b1 = b1_ref[...].astype(f32).reshape(1, F)
        lowest = functools.reduce(jnp.minimum, [_lanes(b1, j) for j in range(nf)])
        split_ref[0] = (jnp.min(lowest) >= MIN_BIAS).astype(jnp.int32)
        loads[-1].start()
        moments([], [0])
        hmxu_refs[-1][z] = normalize(0)
        moments(range(1, early), [])
        moments([], range(1, cycle // 2 + 1))

        w1b = [jnp.concatenate([w1_ref[:, 128 * j:128 * (j + 1)].astype(f32),
                                jnp.where(row < 2, jnp.broadcast_to(_lanes(b1, j), (8, 128)), 0.0)], axis=0)
               for j in range(nf)]
        for j in range(nf):
            seq[pl.ds(8 * j + z, 3)] = _words(w1b[j]).reshape(3, 8, 128)
            seq[W2 + j + z] = _words(w2t_ref[:, 128 * j:128 * (j + 1)])
        w21 = lax.dot_general(w2t_ref[...], jnp.concatenate(w1b, axis=1).astype(bf16),
                              (((1,), (1,)), ((), ())), preferred_element_type=f32)
        diagonal = lax.broadcasted_iota(jnp.int32, (S, S), 0) == lax.broadcasted_iota(jnp.int32, (S, S), 1)
        b2 = jnp.broadcast_to(b2_ref[...].astype(f32).reshape(1, S), (S, S))
        b2 = jnp.sum(jnp.where(diagonal, b2, 0.0), axis=1, keepdims=True)
        acc0_ref[0] = jnp.broadcast_to((2.0 * b2 + w21[:, S:S + 1]) * K, (S, 128))
        acc0_ref[1] = jnp.broadcast_to(2.0 * K * b2, (S, 128))
        high = w21[:, :S].astype(bf16).astype(f32)
        linear = _words(jnp.concatenate(
            [high, jnp.zeros((S, 8), f32), w21[:, :S] - high, jnp.zeros((S, 120 - 2 * S), f32)], axis=1).astype(bf16))

        transposed, stored = {}, set()

        def need_tile(j):
            for i in range(j, min(j + TRANSPOSE_AHEAD + 1, nf)):
                if i not in transposed:
                    src = w1b[i] if j == 0 else pltpu.bitcast(seq[8 * i:8 * i + 3].reshape(S + 8, 128), f32)
                    transposed[i] = jnp.concatenate([src, jnp.zeros((128 - S - 8, 128), f32)], axis=0).T
            if j not in stored:
                stored.add(j)
                seq[pl.ds(8 * j + z, 8)] = _words(transposed[j].astype(bf16)).reshape(8, 8, 128)

        def lhs(i):
            if i == LINEAR:
                seq[LINEAR + z] = linear
            elif i < W2:
                need_tile(i // 8)
            return seq[i]

        def work():
            for n in slots[0]:
                yield from park_h(normalize(1 + n), n, z)
                yield from publish_h(n, z, SETUP_OPS / (sizes[0] * NH))
            for i in range(nvpu):
                need_tile(nf - nvpu + i)
                block = seq[8 * (nf - nvpu + i)]
                column = lambda s: pltpu.bitcast(jnp.broadcast_to(block[:, s:s + 1], (8, 128)), bf16).astype(f32)
                for s in range(8):
                    left, right = column(s), column(8 + s)
                    a11, a21, a12, a22 = left[:8], left[8:], right[:8], right[8:]
                    s1 = a21 + a22
                    s2 = s1 - a11
                    for n, v in enumerate((a11, a12, a12 - s2, a22, s1, s2, a11 - a21)):
                        wcol_ref[i + z, 8 * n + s] = v
                bias = column(S) * K
                wcol_ref[i + z, 56] = bias[:8]
                wcol_ref[i + z, 57] = bias[8:] - bias[:8]
                yield 2 * (S + 1), None, None

        def pace(n, results):
            if n % SETUP_STEP == 0 and n - SETUP_GATE in results:
                seq[SPARE + z] = _words(results[n - SETUP_GATE]())

        target = ramp(SETUP_OPS + 2 * (S + 1) * nvpu, SETUP_START, len(first_period) - SETUP_END)
        acts = run_period(first_period, 0, (cycle - 1, 0), {}, work(), target, z, lhs, SETUP_END, pace)
        for i, key in enumerate(carried):
            carry_ref[i] = acts[key[1:]]
        loads[-1].wait()
        pl.when(split_ref[0] == 0)(without_split)

    def without_split():
        def one_job(job, carry):
            b, cols = job_slice(job)
            moments([b], [])
            moments([], [b])
            rhs = jnp.concatenate([normalize(job), jnp.tile(k_ref[...], (1, TILES))], axis=0)

            def one_tile(j, acc):
                rows = pltpu.bitcast(seq[pl.ds(8 * j, 8)].reshape(64, 128), bf16)
                v = jnp.dot(rows[:, :S + 8], rhs, preferred_element_type=f32)
                g = v * (1.0 + jnp.tanh(v * (C + v * v)))
                return acc + jnp.dot(pltpu.bitcast(seq[W2 + j], bf16), g, preferred_element_type=f32)

            acc = lax.fori_loop(0, nf, one_tile, jnp.tile(acc0_ref[1], (1, TILES)))
            o_ref[b, :, cols] = (acc * (0.5 / K)).astype(o_ref.dtype)
            return carry

        lax.fori_loop(0, njobs, one_job, 0)

    def iteration(step, z, parity):
        mine, other = slots[parity], slots[1 - parity]
        first = 1 + lax.shift_right_logical(step - 1, 1) * cycle + mine[0]
        acts = {key[1:]: carry_ref[i] for i, key in enumerate(carried)}
        batches = lambda last, jobs: [jnp.minimum(lax.shift_right_logical(last, 1) - n, B - 1)
                                      for n in range((jobs + 1) // 2)]
        stats = moments(batches(first - 1 + 2 * cycle, len(other)), batches(first - 1 + cycle + len(mine), len(mine)))

        def prepare_h():
            for n, slot in enumerate(other):
                yield 0, "gate", None
                yield from park_h(normalize(jnp.minimum(first + len(mine) + n, njobs - 1)), slot, z)
                yield from publish_h(slot, z)

        h_work = prepare_h()
        share = -(-(2 + NH) * len(other) // (len(mine) - 1))

        def work(n, total):
            done, issued = 0, 0
            for item in vpu_rows(mine[n], VPU_BLOCKS[parity][n]):
                yield item
                done += item[0]
                if n > 0 and issued < share and done >= (TABLE_FROM + TABLE_SPAN * issued / share) * total:
                    yield next(h_work, (0, None, None))
                    issued += 1
            if n == len(mine) - 1:
                yield from h_work

        def finish_stats(n, _):
            for i, v in enumerate(stats):
                if n == STATS_AT + i * STATS_STEP:
                    seq[pl.ds(SPARE + 1 + z, 2)] = _words(v).reshape(2, 8, 128)

        for n, slot in enumerate(mine):
            plan = periods[slot]
            total = VPU_BLOCKS[parity][n] * (TILES // 2) * sum(COSTS)
            if n == 0:
                body, head = ramp(total - HEAD_OPS, START, len(plan) - END), ramp(HEAD_OPS, START, START + 6)
                target = lambda m: body(m) + head(m)
            else:
                target = ramp(total, 0, len(plan) - END)
            acts = run_period(plan, first + n, (slot, (slot + 1) % cycle), acts, work(n, total), target,
                              z, lambda i: seq[i], END, finish_stats if n == 0 else lambda *_: None)
        for i, key in enumerate(carried):
            carry_ref[i] = acts[key[1:]]

    def loop_body(step, carry):
        z = lax.shift_right_logical(step, 20)
        pl.when(step == 0)(functools.partial(first_job, z))
        split = split_ref[0] > 0
        pl.when(step == steps)(stores[0].start)
        for parity in range(2):
            active = jnp.logical_and(jnp.logical_and(step > 0, split), (step & 1) != parity)
            pl.when(active)(functools.partial(iteration, step, z, parity))
        return carry

    split_ref[0] = 1
    lax.fori_loop(0, steps + 1, loop_body, 0)
    stores[1].start()
    for copy in stores:
        copy.wait()


@jax.jit
def pallas_standalone__mixer_token_mlp__sampling_kernel(
    x: jax.Array,
    w1: jax.Array,
    b1: jax.Array,
    w2: jax.Array,
    b2: jax.Array,
):
    B, tokens, D = x.shape
    F = w1.shape[1]
    nvpu, cycle = max(map(max, VPU_BLOCKS)), sum(map(len, VPU_BLOCKS))
    assert tokens == S and D == 2 * COLS and F % 128 == 0 and F // 128 >= nvpu + 2
    assert (2 * B - 1) % cycle in (0, len(VPU_BLOCKS[0])) and B > cycle
    operands = (x, w1, b1, w2.T, b2)
    in_hbm = pl.BlockSpec(memory_space=pltpu.HBM)
    return pl.pallas_call(
        _kernel,
        out_shape=jax.ShapeDtypeStruct(x.shape, x.dtype),
        in_specs=[in_hbm] * len(operands),
        out_specs=in_hbm,
        scratch_shapes=[pltpu.VMEM(a.shape, a.dtype) for a in operands] + [
            pltpu.VMEM(x.shape, x.dtype),
            pltpu.VMEM((9 * (F // 128) + 4 + 2 * TILES * nvpu, 8, 128), u32),
            pltpu.VMEM((2, S, 128), f32),
            pltpu.VMEM((2 * B + 1, S, 128), f32),
            pltpu.VMEM((nvpu, 60, 8, 128), f32),
            pltpu.VMEM((LAG, S, COLS), f32),
            pltpu.VMEM((8, 128), f32),
            pltpu.VMEM((1 + NH * cycle, 8, 128), f32),
            pltpu.SMEM((1,), jnp.int32),
            pltpu.SemaphoreType.DMA((6,)),
            pltpu.SemaphoreType.DMA((2,)),
        ] + [pltpu.VMEM((64 * NH + 32, 128), f32)] * cycle
          + [pltpu.VMEM((1, S, COLS), f32)] * cycle,
        compiler_params=pltpu.CompilerParams(
            vmem_limit_bytes=64 * 2**20,
            flags={"XLA_TPU_EVENLY_DISTRIBUTE_CRITICAL_NODES": True},
        ),
    )(*operands)
```
